```python
import os as _os
_os.environ.setdefault("JAX_PLATFORMS", "cpu")
import jax
import jax.numpy as jnp

def _softmax(x, axis=-1):
    return jax.nn.softmax(x, axis=axis)
def _gelu(x):
    return jax.nn.gelu(x, approximate=True)
def _silu(x):
    return jax.nn.silu(x)
def _sigmoid(x):
    return jax.nn.sigmoid(x)
def _layernorm(x, axis=-1, eps=1e-5):
    m = jnp.mean(x, axis=axis, keepdims=True)
    v = jnp.var(x, axis=axis, keepdims=True)
    return (x - m) / jnp.sqrt(v + eps)
def _scatter_add(tgt, idx, src, axis=0):
    return tgt.at[idx].add(src)
def _segment_sum(src, seg, n):
    return jax.ops.segment_sum(src, seg, n)
class _Rng:
    def __init__(self, key):
        self._k = key
    def _next(self):
        self._k, sub = jax.random.split(self._k)
        return sub
    def normal(self, shape):
        return jax.random.normal(self._next(), shape, dtype=jnp.bfloat16)
    def randint(self, lo, hi, shape):
        return jax.random.randint(self._next(), shape, lo, hi, dtype=jnp.int32)
    def uniform(self, shape, lo=0.0, hi=1.0):
        return jax.random.uniform(self._next(), shape, jnp.bfloat16, lo, hi)
    def permutation(self, n):
        return jax.random.permutation(self._next(), n)


kernel_name = 'standalone__gqa_softmax__decode'

def setup_inputs():
    _rng = _Rng(jax.random.key(int.from_bytes(__import__("os").urandom(4), "little")))
    _w = (lambda a: (lambda t: t.astype(jnp.bfloat16) if jnp.issubdtype(t.dtype, jnp.floating) else t)(jnp.asarray(a)))
    B, Hq, Hkv, Sq, Sk, D = 2, 32, 32, 1, 8192, 128
    return {
        "q": _w((lambda *s: _rng.normal(s) * 0.8)(B, Hq, Sq, D)),
        "k": _w((lambda *s: _rng.normal(s) * 0.8)(B, Hkv, Sk, D)),
        "v": _w((lambda *s: _rng.normal(s) * 0.05)(B, Hkv, Sk, D)),
    }

def reference(q, k, v):
    B, Hq, Sq, D = q.shape
    Hkv = k.shape[1]
    rep = Hq // Hkv
    k = jnp.repeat(k, rep, axis=1)
    v = jnp.repeat(v, rep, axis=1)
    scale = D ** -0.5
    scores = jnp.einsum("bhqd,bhkd->bhqk", q, k) * scale
    p = _softmax(scores, axis=-1)
    return jnp.einsum("bhqk,bhkd->bhqd", p, v)
```

```python
import jax
import jax.numpy as jnp
import numpy as np
from jax import lax
import jax.experimental.pallas as pl
import jax.experimental.pallas.tpu as pltpu

_CHUNK = 64
_HEADS = 16
_KEYS = 128
_IN_FLIGHT = 2
_LOWEST = float(np.finfo(np.float32).min)


@jax.jit
def pallas_standalone__gqa_softmax__decode_kernel(
    q: jax.Array,
    k: jax.Array,
    v: jax.Array,
):
    B, Hq, Sq, D = q.shape
    _, Hkv, Sk, _ = k.shape
    assert Sq == 1 and Hq == Hkv
    NH = B * Hq
    G, R, C = _HEADS, _KEYS, _CHUNK
    assert NH % G == 0 and Sk % R == 0 and R % C == 0 and R % D == 0
    n_sets = NH // G
    n_steps = n_sets * Sk // R
    n_slots = _IN_FLIGHT + 1
    seg_rows = n_sets * Sk
    step_rows = 2 * G * R
    scale = D ** -0.5

    def position(t, h, c):
        return ((c * G + h) * 2 + t) * C

    def kernel(q_hbm, k_hbm, v_hbm, o_hbm, buf, q32, qs, ms, ls, accs, o32, ob, sems):
        def aligned(x):
            return x if isinstance(x, int) else pl.multiple_of(x, C)

        def start(i, slot):
            for c in range(R // C):
                for h in range(G):
                    for t, src in enumerate((k_hbm, v_hbm)):
                        pltpu.make_async_copy(
                            src.at[pl.ds(aligned(i * R + (h * seg_rows + c * C)), C), :],
                            buf.at[pl.ds(aligned(slot * step_rows + (NH + position(t, h, c))), C), :],
                            sems.at[slot],
                        ).start(priority=t)

        def wait(first_row, n_rows, slot):
            filled = buf.at[pl.ds(aligned(first_row), n_rows), :]
            pltpu.make_async_copy(filled, filled, sems.at[slot]).wait()

        pltpu.make_async_copy(q_hbm, buf.at[pl.ds(0, NH), :], sems.at[0]).start()
        for i in range(_IN_FLIGHT):
            start(i, i)
        ms[...] = jnp.full(ms.shape, _LOWEST, jnp.float32)
        ls[...] = jnp.zeros(ls.shape, jnp.float32)
        accs[...] = jnp.zeros(accs.shape, jnp.float32)
        wait(0, NH + step_rows, 0)

        def gather_q():
            q32[...] = buf[pl.ds(0, NH), :].astype(jnp.float32)
            for s in range(n_sets):
                qs[s] = q32[pl.ds(s, G, stride=n_sets), :].astype(qs.dtype)

        def tile(slot, t, h):
            return jnp.concatenate(
                [buf[pl.ds(aligned(slot * step_rows + (NH + position(t, h, c))), C), :]
                 for c in range(R // C)], axis=0)

        def step(i, slot):
            free = slot + _IN_FLIGHT
            free = jnp.where(free >= n_slots, free - n_slots, free)

            @pl.when(i + _IN_FLIGHT < n_steps)
            def _():
                start(i + _IN_FLIGHT, free)

            pl.when(i == 0)(gather_q)

            st = i // (Sk // R)
            qg = qs[st]
            lane = lax.broadcasted_iota(jnp.int32, (G, R), 0)
            s = None
            for h in range(G):
                r = lax.dot_general(qg, tile(slot, 0, h), (((1,), (1,)), ((), ())),
                                    preferred_element_type=jnp.float32)
                s = r if s is None else jnp.where(lane == h, r, s)
            s = s * scale
            m_old = ms[st]
            m_new = jnp.maximum(m_old, jnp.max(s, axis=1, keepdims=True))
            alpha = jnp.exp(m_old - m_new)
            p = jnp.exp(s - jnp.tile(m_new, (1, R // D)))
            ms[st] = m_new
            ls[st] = jnp.tile(alpha, (1, R // D)) * ls[st] + p
            p = p.astype(v_hbm.dtype)
            lane = lax.broadcasted_iota(jnp.int32, (G, D), 0)
            o = None
            for h in range(G):
                r = jnp.dot(p, tile(slot, 1, h), preferred_element_type=jnp.float32)
                o = r if o is None else jnp.where(lane == h, r, o)
            accs[st] = alpha * accs[st] + o

            slot = jnp.where(slot + 1 == n_slots, 0, slot + 1)

            @pl.when(i + 1 < n_steps)
            def _():
                wait(slot * step_rows + NH, step_rows, slot)

            return slot

        lax.fori_loop(0, n_steps, step, jnp.int32(0))

        for s in range(n_sets):
            o32[pl.ds(s, G, stride=n_sets), :] = accs[s] / jnp.sum(ls[s], axis=1, keepdims=True)
        ob[...] = o32[...].astype(ob.dtype)
        out = pltpu.make_async_copy(ob, o_hbm, sems.at[0])
        out.start()
        out.wait()

    o = pl.pallas_call(
        kernel,
        in_specs=[pl.BlockSpec(memory_space=pltpu.HBM)] * 3,
        out_specs=pl.BlockSpec(memory_space=pltpu.HBM),
        out_shape=jax.ShapeDtypeStruct((NH, D), q.dtype),
        scratch_shapes=[
            pltpu.VMEM((NH + n_slots * step_rows, D), k.dtype),
            pltpu.VMEM((NH, D), jnp.float32),
            pltpu.VMEM((n_sets, G, D), q.dtype),
            pltpu.VMEM((n_sets, G, D), jnp.float32),
            pltpu.VMEM((n_sets, G, R), jnp.float32),
            pltpu.VMEM((n_sets, G, D), jnp.float32),
            pltpu.VMEM((NH, D), jnp.float32),
            pltpu.VMEM((NH, D), q.dtype),
            pltpu.SemaphoreType.DMA((n_slots,)),
        ],
        compiler_params=pltpu.CompilerParams(disable_bounds_checks=True),
        name="gqa_softmax_decode",
    )(q.reshape(NH, D), k.reshape(NH * Sk, D), v.reshape(NH * Sk, D))
    return o.reshape(B, Hq, Sq, D)
```

```python
import jax
import jax.numpy as jnp
import numpy as np
from jax import lax
import jax.experimental.pallas as pl
import jax.experimental.pallas.tpu as pltpu

_CHUNK = 64
_SETS = 4
_V_BEFORE_ISSUE = 29
_LAST_V_SPLIT = 20
_LOWEST = float(np.finfo(np.float32).min)


@jax.jit
def pallas_standalone__gqa_softmax__decode_kernel(
    q: jax.Array,
    k: jax.Array,
    v: jax.Array,
):
    B, Hq, Sq, D = q.shape
    _, Hkv, Sk, _ = k.shape
    assert Sq == 1 and Hq == Hkv
    NH = B * Hq
    C = _CHUNK
    G = NH // _SETS
    L = 2 * G
    assert NH % (16 * _SETS) == 0 and Sk % (4 * C) == 0 and 2 * C == D
    group_rows = 2 * L * C
    n_pairs = Sk // (2 * C)
    n_steps = 2 * n_pairs
    last = n_steps - 1
    head_row = [(n % G * _SETS + n // G * 2) * Sk for n in range(L)]
    span = max(head_row) + C
    scale = D ** -0.5

    def first_row(i, c):
        j = i >> 1
        chunk = 2 * (j % (n_pairs // 2)) + j // (n_pairs // 2)
        return (i & 1) * Sk + (chunk + c * n_pairs) * C

    def aligned(x):
        return x if isinstance(x, int) else pl.multiple_of(x, C)

    def kernel(q_hbm, k_hbm, v_hbm, o_hbm, buf, q32, qs, ms, ls, accs, o32, ob, sems):
        def slots(s, n=1):
            return buf.at[pl.ds(aligned(NH + s * group_rows), n * group_rows), :]

        def copy(t, row, s, n, sem):
            return pltpu.make_async_copy(
                t.at[pl.ds(row, C), :], slots(s).at[pl.ds(n * C, C), :], sems.at[sem])

        def wait(s, first, count, sem):
            filled = slots(s).at[pl.ds(first * C, count * C), :]
            pltpu.make_async_copy(filled, filled, sems.at[sem]).wait()

        def start_group(i, c, s):
            rows = pl.ds(aligned(first_row(i, c)), span)
            ks, vs = k_hbm.at[rows, :], v_hbm.at[rows, :]
            for n in range(L):
                copy(ks, head_row[n], s, n, 2 * s).start(priority=0)
                copy(vs, head_row[n], s, L + n, 2 * s + (n >= _V_BEFORE_ISSUE)).start(priority=1)

        def wait_most(s):
            wait(s, 0, L + _V_BEFORE_ISSUE, 2 * s)

        def wait_rest(s):
            wait(s, L + _V_BEFORE_ISSUE, L - _V_BEFORE_ISSUE, 2 * s + 1)

        end = 2 * (last & 1)
        spare = 2 * (2 - end)

        def start_last_k():
            for n in range(L):
                for c in range(2):
                    copy(k_hbm, first_row(last, c) + head_row[n], end + c, n,
                         2 * (end + c)).start(priority=c)

        def start_last_v():
            for n in range(L):
                for c in range(2):
                    sem = spare if c == 1 and n >= _LAST_V_SPLIT else 2 * (end + c) + 1
                    copy(v_hbm, first_row(last, c) + head_row[n], end + c, L + n,
                         sem).start(priority=c)

        def tile(pair, n):
            return jnp.concatenate(
                [pair[pl.ds(c * group_rows + n * C, C), :] for c in range(2)], axis=0)

        def pick(n, new, old):
            if old is None:
                return new
            return jnp.where(lax.broadcasted_iota(jnp.int32, new.shape, 0) == n % G, new, old)

        def scores(pair, u, st):
            qg = qs[st]
            s = None
            for n in range(u * G, (u + 1) * G):
                s = pick(n, lax.dot_general(qg, tile(pair, n), (((1,), (1,)), ((), ())),
                                            preferred_element_type=jnp.float32), s)
            return s * scale

        def softmax_update(s, st):
            m_old = ms[st]
            m_new = jnp.maximum(m_old, jnp.max(s, axis=1, keepdims=True))
            alpha = jnp.exp(m_old - m_new)
            p = jnp.exp(s - m_new)
            return m_new, alpha * ls[st] + p, p.astype(buf.dtype), alpha

        def weigh(pair, p, n, o):
            return pick(n, jnp.dot(p, tile(pair, L + n), preferred_element_type=jnp.float32), o)

        def gather_q():
            q32[...] = buf[pl.ds(0, NH), :].astype(jnp.float32)
            for st in range(_SETS):
                qs[st] = q32[pl.ds(st, G, stride=_SETS), :].astype(qs.dtype)

        def emit(st, value):
            o32[pl.ds(st, G, stride=_SETS), :] = value

        pltpu.make_async_copy(q_hbm, buf.at[pl.ds(0, NH), :], sems.at[0]).start()
        start_group(0, 0, 0)
        start_group(0, 1, 1)
        ms[...] = jnp.full(ms.shape, _LOWEST, jnp.float32)
        ls[...] = jnp.zeros(ls.shape, jnp.float32)
        accs[...] = jnp.zeros(accs.shape, jnp.float32)
        head = buf.at[pl.ds(0, NH + (L + _V_BEFORE_ISSUE) * C), :]
        pltpu.make_async_copy(head, head, sems.at[0]).wait()

        def step(i, carry):
            cur = 2 * (i & 1)
            nxt = 2 - cur
            pl.when(i + 1 < last)(lambda: start_group(i + 1, 0, nxt))
            pl.when(i + 1 == last)(start_last_k)
            pl.when(i == 0)(gather_q)
            wait_rest(cur)
            wait_most(cur + 1)
            pl.when(i + 1 < last)(lambda: start_group(i + 1, 1, nxt + 1))
            pl.when(i + 1 == last)(start_last_v)
            wait_rest(cur + 1)

            pair = slots(cur, 2)
            sets = [2 * u + (i & 1) for u in range(2)]
            ss = [scores(pair, u, sets[u]) for u in range(2)]
            for u, st in enumerate(sets):
                ms[st], ls[st], p, alpha = softmax_update(ss[u], st)
                o = None
                for n in range(u * G, (u + 1) * G):
                    o = weigh(pair, p, n, o)
                accs[st] = alpha * accs[st] + o

            pl.when(i + 1 < last)(lambda: wait_most(nxt))
            return carry

        lax.fori_loop(0, last, step, 0)

        for st in (0, 2):
            emit(st, accs[st] / jnp.sum(ls[st], axis=1, keepdims=True))
        sets = (1, 3)
        pair = slots(end, 2)
        wait(end, 0, L, 2 * end)
        wait(end + 1, 0, L, 2 * end + 2)
        ss = [scores(pair, u, sets[u]) for u in range(2)]
        state = [softmax_update(ss[0], sets[0])]
        wait(end, L, L, 2 * end + 1)
        wait(end + 1, L, _LAST_V_SPLIT, 2 * end + 3)
        o = [None, None]
        for n in range(G):
            o[0] = weigh(pair, state[0][2], n, o[0])
        state.append(softmax_update(ss[1], sets[1]))
        for n in range(G, _LAST_V_SPLIT):
            o[1] = weigh(pair, state[1][2], n, o[1])
        inv = [1.0 / jnp.sum(l, axis=1, keepdims=True) for _, l, _, _ in state]
        acc = [alpha * accs[st] for st, (_, _, _, alpha) in zip(sets, state)]
        emit(sets[0], (acc[0] + o[0]) * inv[0])
        wait(end + 1, L + _LAST_V_SPLIT, L - _LAST_V_SPLIT, spare)
        for n in range(_LAST_V_SPLIT, L):
            o[1] = weigh(pair, state[1][2], n, o[1])
        emit(sets[1], (acc[1] + o[1]) * inv[1])

        ob[...] = o32[...].astype(ob.dtype)
        out = pltpu.make_async_copy(ob, o_hbm, sems.at[0])
        out.start()
        out.wait()

    o = pl.pallas_call(
        kernel,
        in_specs=[pl.BlockSpec(memory_space=pltpu.HBM)] * 3,
        out_specs=pl.BlockSpec(memory_space=pltpu.HBM),
        out_shape=jax.ShapeDtypeStruct((NH, D), q.dtype),
        scratch_shapes=[
            pltpu.VMEM((NH + 4 * group_rows, D), k.dtype),
            pltpu.VMEM((NH, D), jnp.float32),
            pltpu.VMEM((_SETS, G, D), q.dtype),
            pltpu.VMEM((_SETS, G, 2 * C), jnp.float32),
            pltpu.VMEM((_SETS, G, 2 * C), jnp.float32),
            pltpu.VMEM((_SETS, G, D), jnp.float32),
            pltpu.VMEM((NH, D), jnp.float32),
            pltpu.VMEM((NH, D), q.dtype),
            pltpu.SemaphoreType.DMA((8,)),
        ],
        compiler_params=pltpu.CompilerParams(disable_semaphore_checks=True),
        name="gqa_softmax_decode",
    )(q.reshape(NH, D), k.reshape(NH * Sk, D), v.reshape(NH * Sk, D))
    return o.reshape(B, Hq, Sq, D)
```

```python
import jax
import jax.numpy as jnp
import numpy as np
from jax import lax
import jax.experimental.pallas as pl
import jax.experimental.pallas.tpu as pltpu

_CHUNK = 64
_SETS = 4
_BEFORE_ISSUE = 30
_BEFORE_LAST = 20
_LOWEST = float(np.finfo(np.float32).min)


@jax.jit
def pallas_standalone__gqa_softmax__decode_kernel(
    q: jax.Array,
    k: jax.Array,
    v: jax.Array,
):
    B, Hq, Sq, D = q.shape
    _, Hkv, Sk, _ = k.shape
    assert Sq == 1 and Hq == Hkv
    NH = B * Hq
    C = _CHUNK
    assert NH == 64 and D == 2 * C and Sk % (2 * C) == 0
    G = NH // _SETS
    L = 2 * G
    group_rows = 2 * L * C
    tiles = Sk // (2 * C)
    last = 2 * tiles - 1
    scale = D ** -0.5

    order = [[(thread ^ (n & 1), n & 1, (n >> 1) ^ (n & 1) * 12) for n in range(L)]
             for thread in range(2)]
    position = {item: thread * L + n
                for thread in range(2) for n, item in enumerate(order[thread])}

    def head_row(u, row):
        return (row * _SETS + 2 * u) * Sk

    def first_row(i, c):
        return i // tiles * Sk + (2 * (i % tiles) + c) * C

    def aligned(x):
        return x if isinstance(x, int) else pl.multiple_of(x, C)

    def kernel(q_hbm, k_hbm, v_hbm, o_hbm, buf, q32, qs, ms, ls, accs, o32, ob, sems):
        def slots(s, n=1):
            return buf.at[pl.ds(aligned(NH + s * group_rows), n * group_rows), :]

        def start(s, source, split):
            for n in range(L):
                for thread in range(2):
                    pltpu.make_async_copy(
                        source(*order[thread][n]),
                        slots(s).at[pl.ds((thread * L + n) * C, C), :],
                        sems.at[2 * s + (thread == 1 and n >= split)],
                    ).start(priority=thread)

        def wait_most(s, split):
            filled = slots(s).at[pl.ds(0, (L + split) * C), :]
            pltpu.make_async_copy(filled, filled, sems.at[2 * s]).wait()

        def wait_rest(s, split):
            filled = slots(s).at[pl.ds((L + split) * C, (L - split) * C), :]
            pltpu.make_async_copy(filled, filled, sems.at[2 * s + 1]).wait()

        def start_group(i, c, s):
            rows = pl.ds(aligned(first_row(i, c)), head_row(1, G - 1) + C)
            kv = k_hbm.at[rows, :], v_hbm.at[rows, :]
            start(s, lambda t, u, row: kv[t].at[pl.ds(head_row(u, row), C), :], _BEFORE_ISSUE)

        end = 2 * (last & 1)

        def start_last(t):
            src = (k_hbm, v_hbm)[t]
            start(end + t,
                  lambda c, u, row: src.at[pl.ds(first_row(last, c) + head_row(u, row), C), :],
                  (L, _BEFORE_LAST)[t])

        def tile(pair, t, u, row, swapped):
            places = [(t, position[c, u, row]) if swapped else (c, position[t, u, row])
                      for c in range(2)]
            return jnp.concatenate(
                [pair[pl.ds(g * group_rows + n * C, C), :] for g, n in places], axis=0)

        def pick(row, new, old):
            if old is None:
                return new
            return jnp.where(lax.broadcasted_iota(jnp.int32, new.shape, 0) == row, new, old)

        def scores(pair, u, st, swapped=False):
            qg = qs[st]
            s = None
            for row in range(G):
                s = pick(row, lax.dot_general(
                    qg, tile(pair, 0, u, row, swapped), (((1,), (1,)), ((), ())),
                    preferred_element_type=jnp.float32), s)
            return s * scale

        def softmax_update(s, st):
            m_old = ms[st]
            m_new = jnp.maximum(m_old, jnp.max(s, axis=1, keepdims=True))
            alpha = jnp.exp(m_old - m_new)
            p = jnp.exp(s - m_new)
            return m_new, alpha * ls[st] + p, p.astype(buf.dtype), alpha

        def weigh(pair, p, u, rows, o=None, swapped=False):
            for row in rows:
                o = pick(row, jnp.dot(p, tile(pair, 1, u, row, swapped),
                                      preferred_element_type=jnp.float32), o)
            return o

        def gather_q():
            q32[...] = buf[pl.ds(0, NH), :].astype(jnp.float32)
            for st in range(_SETS):
                qs[st] = q32[pl.ds(st, G, stride=_SETS), :].astype(qs.dtype)

        def emit(st, value):
            o32[pl.ds(st, G, stride=_SETS), :] = value

        pltpu.make_async_copy(q_hbm, buf.at[pl.ds(0, NH), :], sems.at[0]).start()
        start_group(0, 0, 0)
        start_group(0, 1, 1)
        ms[...] = jnp.full(ms.shape, _LOWEST, jnp.float32)
        ls[...] = jnp.zeros(ls.shape, jnp.float32)
        accs[...] = jnp.zeros(accs.shape, jnp.float32)
        filled = buf.at[pl.ds(0, NH + (L + _BEFORE_ISSUE) * C), :]
        pltpu.make_async_copy(filled, filled, sems.at[0]).wait()

        def step(i, carry):
            cur = 2 * (i & 1)
            nxt = 2 - cur
            pl.when(i + 1 < last)(lambda: start_group(i + 1, 0, nxt))
            pl.when(i + 1 == last)(lambda: start_last(0))
            pl.when(i == 0)(gather_q)
            wait_rest(cur, _BEFORE_ISSUE)
            wait_most(cur + 1, _BEFORE_ISSUE)
            pl.when(i + 1 < last)(lambda: start_group(i + 1, 1, nxt + 1))
            pl.when(i + 1 == last)(lambda: start_last(1))
            wait_rest(cur + 1, _BEFORE_ISSUE)

            pair = slots(cur, 2)
            sets = [2 * u + i // tiles for u in range(2)]
            ss = [scores(pair, u, sets[u]) for u in range(2)]
            for u, st in enumerate(sets):
                ms[st], ls[st], p, alpha = softmax_update(ss[u], st)
                accs[st] = alpha * accs[st] + weigh(pair, p, u, range(G))

            pl.when(i + 1 < last)(lambda: wait_most(nxt, _BEFORE_ISSUE))
            return carry

        lax.fori_loop(0, last, step, 0)

        for st in (0, 2):
            emit(st, accs[st] / jnp.sum(ls[st], axis=1, keepdims=True))
        sets = (1, 3)
        pair = slots(end, 2)
        early = [[r for _, w, r in order[1][:_BEFORE_LAST] if w == u] for u in range(2)]
        late = [[r for _, w, r in order[1][_BEFORE_LAST:] if w == u] for u in range(2)]
        wait_most(end, L)
        ss = [scores(pair, u, sets[u], swapped=True) for u in range(2)]
        state = [softmax_update(ss[0], sets[0])]
        wait_most(end + 1, _BEFORE_LAST)
        o = [weigh(pair, state[0][2], 0, early[0], swapped=True)]
        state.append(softmax_update(ss[1], sets[1]))
        o.append(weigh(pair, state[1][2], 1, early[1], swapped=True))
        inv = [1.0 / jnp.sum(l, axis=1, keepdims=True) for _, l, _, _ in state]
        acc = [alpha * accs[st] for st, (_, _, _, alpha) in zip(sets, state)]
        wait_rest(end + 1, _BEFORE_LAST)
        for u, st in enumerate(sets):
            emit(st, (acc[u] + weigh(pair, state[u][2], u, late[u], o[u], swapped=True)) * inv[u])

        ob[...] = o32[...].astype(ob.dtype)
        out = pltpu.make_async_copy(ob, o_hbm, sems.at[0])
        out.start()
        out.wait()

    o = pl.pallas_call(
        kernel,
        in_specs=[pl.BlockSpec(memory_space=pltpu.HBM)] * 3,
        out_specs=pl.BlockSpec(memory_space=pltpu.HBM),
        out_shape=jax.ShapeDtypeStruct((NH, D), q.dtype),
        scratch_shapes=[
            pltpu.VMEM((NH + 4 * group_rows, D), k.dtype),
            pltpu.VMEM((NH, D), jnp.float32),
            pltpu.VMEM((_SETS, G, D), q.dtype),
            pltpu.VMEM((_SETS, G, 2 * C), jnp.float32),
            pltpu.VMEM((_SETS, G, 2 * C), jnp.float32),
            pltpu.VMEM((_SETS, G, D), jnp.float32),
            pltpu.VMEM((NH, D), jnp.float32),
            pltpu.VMEM((NH, D), q.dtype),
            pltpu.SemaphoreType.DMA((8,)),
        ],
        compiler_params=pltpu.CompilerParams(disable_semaphore_checks=True),
        name="gqa_softmax_decode",
    )(q.reshape(NH, D), k.reshape(NH * Sk, D), v.reshape(NH * Sk, D))
    return o.reshape(B, Hq, Sq, D)
```
